```python
import os as _os
_os.environ.setdefault("JAX_PLATFORMS", "cpu")
import jax
import jax.numpy as jnp

def _softmax(x, axis=-1):
    return jax.nn.softmax(x, axis=axis)
def _gelu(x):
    return jax.nn.gelu(x, approximate=True)
def _silu(x):
    return jax.nn.silu(x)
def _sigmoid(x):
    return jax.nn.sigmoid(x)
def _layernorm(x, axis=-1, eps=1e-5):
    m = jnp.mean(x, axis=axis, keepdims=True)
    v = jnp.var(x, axis=axis, keepdims=True)
    return (x - m) / jnp.sqrt(v + eps)
def _scatter_add(tgt, idx, src, axis=0):
    return tgt.at[idx].add(src)
def _segment_sum(src, seg, n):
    return jax.ops.segment_sum(src, seg, n)
class _Rng:
    def __init__(self, key):
        self._k = key
    def _next(self):
        self._k, sub = jax.random.split(self._k)
        return sub
    def normal(self, shape):
        return jax.random.normal(self._next(), shape, dtype=jnp.bfloat16)
    def randint(self, lo, hi, shape):
        return jax.random.randint(self._next(), shape, lo, hi, dtype=jnp.int32)
    def uniform(self, shape, lo=0.0, hi=1.0):
        return jax.random.uniform(self._next(), shape, jnp.bfloat16, lo, hi)
    def permutation(self, n):
        return jax.random.permutation(self._next(), n)


kernel_name = 'standalone__mha_softmax__near_ridge'

def setup_inputs():
    _rng = _Rng(jax.random.key(int.from_bytes(__import__("os").urandom(4), "little")))
    _w = (lambda a: (lambda t: t.astype(jnp.bfloat16) if jnp.issubdtype(t.dtype, jnp.floating) else t)(jnp.asarray(a)))
    B, H, Sq, Sk, D = 8, 32, 384, 512, 128
    return {
        "q": _w((lambda *s: _rng.normal(s) * 0.4)(B, H, Sq, D)),
        "k": _w((lambda *s: _rng.normal(s) * 0.4)(B, H, Sk, D)),
        "v": _w((lambda *s: _rng.normal(s) * 0.05)(B, H, Sk, D)),
    }

def reference(q, k, v):
    scale = q.shape[-1] ** -0.5
    scores = jnp.einsum("bhqd,bhkd->bhqk", q, k) * scale
    p = _softmax(scores, axis=-1)
    return jnp.einsum("bhqk,bhkd->bhqd", p, v)
```

```python
import jax
import jax.numpy as jnp
import jax.experimental.pallas as pl
import jax.experimental.pallas.tpu as pltpu

_LOG2E = 1.4426950408889634


@jax.jit
def pallas_standalone__mha_softmax__near_ridge_kernel(
    q: jax.Array,
    k: jax.Array,
    v: jax.Array,
):
    B, H, Sq, D = q.shape
    Sk = k.shape[2]
    BH = B * H
    G = 8
    R = 6
    W = 26
    n = BH // G
    c = (D ** -0.5) * _LOG2E

    q3 = q.reshape(BH, Sq, D)
    k3 = k.reshape(BH, Sk, D)
    v3 = v.reshape(BH, Sk, D)

    def kernel(q_hbm, k_hbm, v_hbm, o_hbm, qb, kb, vb, ob, sem_in, sem_out):
        def in_copies(i, slot):
            return [
                pltpu.make_async_copy(q_hbm.at[pl.ds(i * G, G)], qb.at[slot], sem_in.at[slot]),
                pltpu.make_async_copy(k_hbm.at[pl.ds(i * G, G)], kb.at[slot], sem_in.at[R + slot]),
                pltpu.make_async_copy(v_hbm.at[pl.ds(i * G, G)], vb.at[slot], sem_in.at[2 * R + slot]),
            ]

        def out_copy(i):
            return pltpu.make_async_copy(
                ob.at[pl.ds(i * G, G)], o_hbm.at[pl.ds(i * G, G)], sem_out.at[0])

        for j in range(R - 1):
            for cp in in_copies(j, j):
                cp.start()

        def body(i, carry):
            slot = i % R

            @pl.when(i + R - 1 < n)
            def _():
                for cp in in_copies(i + R - 1, (i + R - 1) % R):
                    cp.start()

            for cp in in_copies(i, slot):
                cp.wait()

            for h in range(G):
                s = jax.lax.dot_general(
                    qb[slot, h], kb[slot, h], (((1,), (1,)), ((), ())),
                    preferred_element_type=jnp.float32)
                m = jnp.max(s, axis=-1, keepdims=True)
                p = jnp.exp2((s - m) * c)
                l = jnp.sum(p, axis=-1, keepdims=True)
                o = jnp.dot(p.astype(jnp.bfloat16), vb[slot, h],
                            preferred_element_type=jnp.float32)
                r = pl.reciprocal(l, approx=True)
                r = r * (2.0 - l * r)
                ob[i * G + h] = (o * r).astype(ob.dtype)

            @pl.when(i == W)
            def _():
                def wb(j, c2):
                    out_copy(j).start()
                    return c2
                jax.lax.fori_loop(0, W + 1, wb, 0)

            @pl.when(i > W)
            def _():
                out_copy(i).start()

            return carry

        jax.lax.fori_loop(0, n, body, 0)
        pltpu.make_async_copy(ob, ob, sem_out.at[0]).wait()

    out = pl.pallas_call(
        kernel,
        in_specs=[pl.BlockSpec(memory_space=pl.ANY)] * 3,
        out_specs=pl.BlockSpec(memory_space=pl.ANY),
        out_shape=jax.ShapeDtypeStruct((BH, Sq, D), q.dtype),
        scratch_shapes=[
            pltpu.VMEM((R, G, Sq, D), q.dtype),
            pltpu.VMEM((R, G, Sk, D), k.dtype),
            pltpu.VMEM((R, G, Sk, D), v.dtype),
            pltpu.VMEM((BH, Sq, D), q.dtype),
            pltpu.SemaphoreType.DMA((3 * R,)),
            pltpu.SemaphoreType.DMA((1,)),
        ],
        compiler_params=pltpu.CompilerParams(vmem_limit_bytes=100 * 1024 * 1024),
    )(q3, k3, v3)
    return out.reshape(B, H, Sq, D)
```

```python
import jax
import jax.numpy as jnp
import jax.experimental.pallas as pl
import jax.experimental.pallas.tpu as pltpu

_LOG2E = 1.4426950408889634

_RING = 12
_PRO = 5
_EXTRA = 4
_FULL = 2
_PIECES = 20
_PROWS = 16
_S_ROWS = (0,)
_O_ROWS = (0, 192)
_WSTART = 24
_WFIRST = 14
_WROWS = 128


def _zero_after(x):
    bits = jax.lax.bitcast_convert_type(x, jnp.int32)
    return jax.lax.shift_right_logical(bits & 0x7FFFFFFF, 31)


@jax.jit
def pallas_standalone__mha_softmax__near_ridge_kernel(
    q: jax.Array,
    k: jax.Array,
    v: jax.Array,
):
    B, H, Sq, D = q.shape
    Sk = k.shape[2]
    G, n, R = B, H, _RING
    c = (D ** -0.5) * _LOG2E

    n_ev = len(_S_ROWS) + len(_O_ROWS)
    ev_iter = n_ev * G
    ev_total = (n - _FULL) * _PIECES
    vrows0 = _PIECES * _PROWS
    n_wr = Sq // _WROWS

    assert vrows0 <= Sk and _PIECES <= ev_iter and Sq % _WROWS == 0
    assert _FULL <= _PRO <= R and _WFIRST <= _WSTART + 1 <= n - 2
    for e in range(ev_total):
        grp, it = _FULL + e // _PIECES, e // ev_iter
        assert it < grp <= it + R - 1
    for it in range(n):
        issued = min(_PRO + (it + 1) + (it + 1) // _EXTRA, n)
        assert issued >= min(it + 2, n) and issued - 1 - R <= it

    def kernel(q_hbm, k_hbm, v_hbm, o_hbm, qb, kb, vb, ob, sem_in, sem_out):
        def q_copy(g, slot):
            return pltpu.make_async_copy(q_hbm.at[:, g], qb.at[slot], sem_in.at[slot])

        def k_copy(g, slot):
            return pltpu.make_async_copy(k_hbm.at[:, g], kb.at[slot], sem_in.at[R + slot])

        def v_copy(g, slot):
            return pltpu.make_async_copy(v_hbm.at[:, g], vb.at[slot], sem_in.at[2 * R + slot])

        def v_rest_copy(g, slot):
            rows = pl.ds(vrows0, Sk - vrows0)
            return pltpu.make_async_copy(
                v_hbm.at[:, g, rows], vb.at[slot, :, rows], sem_in.at[2 * R + slot])

        def start_bulk_reads(g, slot, whole_v=False):
            q_copy(g, slot).start(priority=1)
            k_copy(g, slot).start(priority=1)
            if whole_v:
                v_copy(g, slot).start(priority=1)
            elif vrows0 < Sk:
                v_rest_copy(g, slot).start(priority=1)

        def start_writes(g):
            for r in range(n_wr):
                rows = pl.ds(r * _WROWS, _WROWS)
                pltpu.make_async_copy(
                    ob.at[:, g, rows], o_hbm.at[:, g, rows], sem_out.at[0]
                ).start(priority=1)

        def start_writes_range(lo, hi):
            def one(g, carry):
                start_writes(g)
                return carry
            jax.lax.fori_loop(lo, hi, one, 0)

        for g in range(_PRO):
            start_bulk_reads(g, g, whole_v=(g < _FULL))

        def body(i, slot):
            def small_v_read(idx, zero):
                e = i * ev_iter + idx
                g0 = jax.lax.div(e, _PIECES)
                grp = _FULL + g0
                row = pl.multiple_of((e - g0 * _PIECES) * _PROWS + zero * _PROWS, _PROWS)
                gs = jax.lax.rem(grp, R)

                @pl.when(e < ev_total)
                def _():
                    rows = pl.ds(row, _PROWS)
                    pltpu.make_async_copy(
                        v_hbm.at[:, grp, rows], vb.at[gs, :, rows], sem_in.at[2 * R + gs]
                    ).start(priority=0)

            q_copy(i, slot).wait()
            k_copy(i, slot).wait()
            v_copy(i, slot).wait()

            @pl.when(i > _WSTART + 2)
            def _():
                start_writes(i - 1)

            def scores(h):
                s = jax.lax.dot_general(
                    qb[slot, h], kb[slot, h], (((1,), (1,)), ((), ())),
                    preferred_element_type=jnp.float32)
                for t, row in enumerate(_S_ROWS):
                    small_v_read(h * n_ev + t, _zero_after(s[row, 0]))
                return s

            s = scores(0)
            for h in range(G):
                s_next = scores(h + 1) if h + 1 < G else None
                m = jnp.max(s, axis=-1, keepdims=True)
                p = jnp.exp2((s - m) * c)
                l = jnp.sum(p, axis=-1, keepdims=True)
                o = jnp.dot(p.astype(jnp.bfloat16), vb[slot, h],
                            preferred_element_type=jnp.float32)
                for t, row in enumerate(_O_ROWS):
                    small_v_read(h * n_ev + len(_S_ROWS) + t, _zero_after(o[row, 0]))
                r = pl.reciprocal(l, approx=True)
                r = r * (2.0 - l * r)
                ob[h, i] = (o * r).astype(ob.dtype)
                s = s_next

            ix = jax.lax.div(i, _EXTRA)
            g1 = _PRO + i + ix

            @pl.when(g1 < n)
            def _():
                start_bulk_reads(g1, jax.lax.rem(g1, R))

            @pl.when(jnp.logical_and(i - ix * _EXTRA == _EXTRA - 1, g1 + 1 < n))
            def _():
                start_bulk_reads(g1 + 1, jax.lax.rem(g1 + 1, R))

            @pl.when(i == _WSTART)
            def _():
                start_writes_range(0, _WFIRST)

            @pl.when(i == _WSTART + 1)
            def _():
                start_writes_range(_WFIRST, _WSTART + 2)

            return jnp.where(slot == R - 1, 0, slot + 1)

        jax.lax.fori_loop(0, n, body, 0)
        start_writes(n - 1)
        pltpu.make_async_copy(ob, ob, sem_out.at[0]).wait()

    return pl.pallas_call(
        kernel,
        in_specs=[pl.BlockSpec(memory_space=pl.ANY)] * 3,
        out_specs=pl.BlockSpec(memory_space=pl.ANY),
        out_shape=jax.ShapeDtypeStruct((B, H, Sq, D), q.dtype),
        scratch_shapes=[
            pltpu.VMEM((R, G, Sq, D), q.dtype),
            pltpu.VMEM((R, G, Sk, D), k.dtype),
            pltpu.VMEM((R, G, Sk, D), v.dtype),
            pltpu.VMEM((B, H, Sq, D), q.dtype),
            pltpu.SemaphoreType.DMA((3 * R,)),
            pltpu.SemaphoreType.DMA((1,)),
        ],
        compiler_params=pltpu.CompilerParams(
            vmem_limit_bytes=100 * 1024 * 1024,
            disable_bounds_checks=True,
        ),
    )(q, k, v)
```

```python
import jax
import jax.numpy as jnp
import jax.experimental.pallas as pl
import jax.experimental.pallas.tpu as pltpu

_LOG2E = 1.4426950408889634

_RING = 12
_PRO = 5
_EXTRA = 4
_FULL = 2
_PROWS = 16
_EVENTS = 5
_SPACING = 11
_WSTART = 24
_WFIRST = 14
_WROWS = 128


def _zero_after(x):
    bits = jax.lax.bitcast_convert_type(x, jnp.uint32)
    return jax.lax.shift_right_logical(bits & jnp.uint32(0x7FFFFFFF), jnp.uint32(31))


def _zero_later(z):
    for _ in range(_SPACING):
        z = jax.lax.div(jnp.uint32(7), z + jnp.uint32(1000))
    return z


@jax.jit
def pallas_standalone__mha_softmax__near_ridge_kernel(
    q: jax.Array,
    k: jax.Array,
    v: jax.Array,
):
    B, H, Sq, D = q.shape
    Sk = k.shape[2]
    G, n, R = B, H, _RING
    c = (D ** -0.5) * _LOG2E

    pieces = Sk // _PROWS
    ev_iter = _EVENTS * G
    ev_total = (n - _FULL) * pieces
    n_wr = Sq // _WROWS

    assert Sk % _PROWS == 0 and pieces <= ev_iter and Sq % _WROWS == 0
    assert _FULL <= _PRO <= R and _WFIRST <= _WSTART + 1 <= n - 2
    for e in range(ev_total):
        grp, it = _FULL + e // pieces, e // ev_iter
        assert it < grp <= it + R - 1
    for it in range(n):
        issued = min(_PRO + (it + 1) + (it + 1) // _EXTRA, n)
        assert issued >= min(it + 2, n) and issued - 1 - R <= it

    def kernel(q_hbm, k_hbm, v_hbm, o_hbm, qb, kb, vb, ob, sem_in, sem_out):
        def q_copy(g, slot):
            return pltpu.make_async_copy(q_hbm.at[:, g], qb.at[slot], sem_in.at[slot])

        def k_copy(g, slot):
            return pltpu.make_async_copy(k_hbm.at[:, g], kb.at[slot], sem_in.at[R + slot])

        def v_copy(g, slot):
            return pltpu.make_async_copy(v_hbm.at[:, g], vb.at[slot], sem_in.at[2 * R + slot])

        def start_qk_reads(g, slot):
            q_copy(g, slot).start(priority=1)
            k_copy(g, slot).start(priority=1)

        def start_writes(g):
            for r in range(n_wr):
                rows = pl.ds(r * _WROWS, _WROWS)
                pltpu.make_async_copy(
                    ob.at[:, g, rows], o_hbm.at[:, g, rows], sem_out.at[0]
                ).start(priority=1)

        def start_writes_range(lo, hi):
            def one(g, carry):
                start_writes(g)
                return carry
            jax.lax.fori_loop(lo, hi, one, 0)

        for g in range(_PRO):
            start_qk_reads(g, g)
            if g < _FULL:
                v_copy(g, g).start(priority=1)

        def body(i, slot):
            def small_v_read(idx, zero):
                e = i * ev_iter + idx
                g0 = jax.lax.div(e, pieces)
                grp = _FULL + g0
                piece = jnp.clip(e - g0 * pieces + zero.astype(jnp.int32), 0, pieces - 1)
                row = pl.multiple_of(piece * _PROWS, _PROWS)
                gs = jax.lax.rem(grp, R)

                @pl.when(e < ev_total)
                def _():
                    rows = pl.ds(row, _PROWS)
                    pltpu.make_async_copy(
                        v_hbm.at[:, grp, rows], vb.at[gs, :, rows], sem_in.at[2 * R + gs]
                    ).start(priority=0)

            q_copy(i, slot).wait()
            k_copy(i, slot).wait()
            v_copy(i, slot).wait()

            @pl.when(i > _WSTART + 2)
            def _():
                start_writes(i - 1)

            for h in range(G):
                s = jax.lax.dot_general(
                    qb[slot, h], kb[slot, h], (((1,), (1,)), ((), ())),
                    preferred_element_type=jnp.float32)
                m = jnp.max(s, axis=-1, keepdims=True)
                p = jnp.exp2((s - m) * c)
                l = jnp.sum(p, axis=-1, keepdims=True)
                o = jnp.dot(p.astype(jnp.bfloat16), vb[slot, h],
                            preferred_element_type=jnp.float32)
                zero = _zero_after(o[0, 0])
                for t in range(_EVENTS):
                    if t:
                        zero = _zero_later(zero)
                    small_v_read(h * _EVENTS + t, zero)
                r = pl.reciprocal(l, approx=True)
                r = r * (2.0 - l * r)
                ob[h, i] = (o * r).astype(ob.dtype)

            ix = jax.lax.div(i, _EXTRA)
            g1 = _PRO + i + ix

            @pl.when(g1 < n)
            def _():
                start_qk_reads(g1, jax.lax.rem(g1, R))

            @pl.when(jnp.logical_and(i - ix * _EXTRA == _EXTRA - 1, g1 + 1 < n))
            def _():
                start_qk_reads(g1 + 1, jax.lax.rem(g1 + 1, R))

            @pl.when(i == _WSTART)
            def _():
                start_writes_range(0, _WFIRST)

            @pl.when(i == _WSTART + 1)
            def _():
                start_writes_range(_WFIRST, _WSTART + 2)

            return jnp.where(slot == R - 1, 0, slot + 1)

        jax.lax.fori_loop(0, n, body, 0)
        start_writes(n - 1)
        pltpu.make_async_copy(ob, ob, sem_out.at[0]).wait()

    return pl.pallas_call(
        kernel,
        in_specs=[pl.BlockSpec(memory_space=pl.ANY)] * 3,
        out_specs=pl.BlockSpec(memory_space=pl.ANY),
        out_shape=jax.ShapeDtypeStruct((B, H, Sq, D), q.dtype),
        scratch_shapes=[
            pltpu.VMEM((R, G, Sq, D), q.dtype),
            pltpu.VMEM((R, G, Sk, D), k.dtype),
            pltpu.VMEM((R, G, Sk, D), v.dtype),
            pltpu.VMEM((B, H, Sq, D), q.dtype),
            pltpu.SemaphoreType.DMA((3 * R,)),
            pltpu.SemaphoreType.DMA((1,)),
        ],
        compiler_params=pltpu.CompilerParams(
            vmem_limit_bytes=100 * 1024 * 1024,
            disable_bounds_checks=True,
        ),
    )(q, k, v)
```
